```python
import jax
import jax.numpy as jnp

def _softmax(x, axis=-1):
    return jax.nn.softmax(x, axis=axis)
def _gelu(x):
    return jax.nn.gelu(x, approximate=True)
def _silu(x):
    return jax.nn.silu(x)
def _sigmoid(x):
    return jax.nn.sigmoid(x)
def _layernorm(x, axis=-1, eps=1e-5):
    m = jnp.mean(x, axis=axis, keepdims=True)
    v = jnp.var(x, axis=axis, keepdims=True)
    return (x - m) / jnp.sqrt(v + eps)
def _scatter_add(tgt, idx, src, axis=0):
    return tgt.at[idx].add(src)
def _segment_sum(src, seg, n):
    return jax.ops.segment_sum(src, seg, n)
class _Rng:
    def __init__(self, key):
        self._k = key
    def _next(self):
        self._k, sub = jax.random.split(self._k)
        return sub
    def normal(self, shape):
        return jax.random.normal(self._next(), shape, dtype=jnp.bfloat16)
    def randint(self, lo, hi, shape):
        return jax.random.randint(self._next(), shape, lo, hi, dtype=jnp.int32)
    def uniform(self, shape, lo=0.0, hi=1.0):
        return jax.random.uniform(self._next(), shape, jnp.bfloat16, lo, hi)
    def permutation(self, n):
        return jax.random.permutation(self._next(), n)


kernel_name = 'recurrent_scan__linear_kernel_hedgehog__dense_activation_relu__prompt'

def _fwd_setup_inputs():
    _rng = _Rng(jax.random.key(int.from_bytes(__import__("os").urandom(4), "little")))
    _w = (lambda a: (lambda t: t.astype(jnp.bfloat16) if jnp.issubdtype(t.dtype, jnp.floating) else t)(jnp.asarray(a)))
    def _A_setup():
        B, S, D, H = 1, 2048, 1024, 32
        Dh = D // H
        return {
            "x": _w((lambda *s: _rng.normal(s) * 0.05)(B, S, D)),
            "wqkv": _w((lambda *s: _rng.normal(s) * 0.05)(D, 3 * D)),
            "w_phi": _w((lambda *s: _rng.normal(s) * 0.05)(H, Dh, Dh) * (Dh ** -0.5)),
            "wo": _w((lambda *s: _rng.normal(s) * 0.05)(D, D)),
        }
    _A_in = _A_setup()

    def _B_setup():
        B, S, D, Dff = 1, 2048, 1024, 3584
        return {
            "x": _w((lambda *s: _rng.normal(s) * 0.05)(B, S, D)),
            "w1": _w((lambda *s: _rng.normal(s) * 0.05)(D, Dff)),
            "w2": _w((lambda *s: _rng.normal(s) * 0.05)(Dff, D)),
        }
    _B_in = _B_setup()

    return {
        "A_x": _A_in["x"],
        "A_wqkv": _A_in["wqkv"],
        "A_w_phi": _A_in["w_phi"],
        "A_wo": _A_in["wo"],
        "B_x": _B_in["x"],
        "B_w1": _B_in["w1"],
        "B_w2": _B_in["w2"],
    }

def _fwd_reference(A_x, A_wqkv, A_w_phi, A_wo, B_x, B_w1, B_w2):
    def _A_ref(x, wqkv, w_phi, wo):
        B, S, D = x.shape
        H = 32; Dh = D // H
        qkv = (lambda x, *d: x.transpose(*d))((x @ wqkv).reshape(B, S, 3, H, Dh), 2, 0, 3, 1, 4)
        q, k, v = qkv[0], qkv[1], qkv[2]
        pq = jnp.einsum("bhsd,hdf->bhsf", q, w_phi)
        pk = jnp.einsum("bhsd,hdf->bhsf", k, w_phi)
        phi_q = jnp.concatenate([_softmax(pq, axis=-1), _softmax(-pq, axis=-1)], axis=-1)
        phi_k = jnp.concatenate([_softmax(pk, axis=-1), _softmax(-pk, axis=-1)], axis=-1)
        kv = jnp.einsum("bhsf,bhsd->bhfd", phi_k, v)
        z  = jnp.einsum("bhsf->bhf", phi_k)
        num = jnp.einsum("bhqf,bhfd->bhqd", phi_q, kv)
        den = jnp.einsum("bhqf,bhf->bhq", phi_q, z)[..., None] + 1e-6
        o = num / den
        return (lambda x, *d: x.transpose(*d))(o, 0, 2, 1, 3).reshape(B, S, D) @ wo

    def _B_ref(x, w1, w2):
        h = jnp.einsum("bsd,df->bsf", x, w1)
        zero = jnp.zeros_like(h)
        h = jnp.maximum(h, zero)
        return jnp.einsum("bsf,fd->bsd", h, w2)

    x = A_x
    xn = _layernorm(x, axis=-1)
    s = _A_ref(xn, A_wqkv, A_w_phi, A_wo)
    g = _silu(_B_ref(xn, B_w1, B_w2))
    return x + s * g


def setup_inputs():
    _inp = _fwd_setup_inputs()
    _gk = jax.random.fold_in(jax.random.key(int.from_bytes(__import__("os").urandom(4), "little")), 2**31 - 1)
    _shapes = [[1, 2048, 1024]]
    _dtypes = ['bfloat16']
    _gks = jax.random.split(_gk, len(_shapes))
    _gs = [jax.random.normal(k, s, dtype=jnp.dtype(d)) * 0.05 for k, s, d in zip(_gks, _shapes, _dtypes)]
    _inp["grad_out"] = _gs[0]
    return _inp

def reference(A_x, A_wqkv, A_w_phi, A_wo, B_w1, B_w2, B_x, grad_out):
    _const = dict(B_x=B_x)
    def _f(*_d):
        return _fwd_reference(**{'A_x': _d[0], 'A_wqkv': _d[1], 'A_w_phi': _d[2], 'A_wo': _d[3], 'B_w1': _d[4], 'B_w2': _d[5], **_const})
    _out, _vjp = jax.vjp(_f, A_x, A_wqkv, A_w_phi, A_wo, B_w1, B_w2)
    _grads = _vjp(grad_out)
    _out0 = jnp.asarray(_out)
    return (_out0, *[jnp.asarray(_g) for _g in _grads])
```

```python
import jax
import jax.numpy as jnp
from jax import lax
import jax.experimental.pallas as pl
import jax.experimental.pallas.tpu as pltpu

S, D, F, H, DH = 2048, 1024, 3584, 32, 32
G = 8
T = 256
NT = S // T
FC = 512
NC = F // FC
KT = 512
XR = 32
BF, F32 = jnp.bfloat16, jnp.float32


def _nn(a, b):
    return lax.dot_general(a, b, (((1,), (0,)), ((), ())), preferred_element_type=F32)


def _nt(a, b):
    return lax.dot_general(a, b, (((1,), (1,)), ((), ())), preferred_element_type=F32)


def _tn(a, b):
    return lax.dot_general(a, b, (((0,), (0,)), ((), ())), preferred_element_type=F32)


def _iota(shape, axis):
    return lax.broadcasted_iota(jnp.int32, shape, axis)


def _layernorm(x):
    xc = x - jnp.mean(x, axis=-1, keepdims=True)
    rstd = lax.rsqrt(jnp.mean(xc * xc, axis=-1, keepdims=True) + 1e-5)
    return xc * rstd, rstd


def _features(p):
    n = p.shape[1]
    p = p.reshape(4, DH, n)
    e = jnp.concatenate([jnp.exp(p - jnp.max(p, axis=1, keepdims=True)),
                         jnp.exp(jnp.min(p, axis=1, keepdims=True) - p)], axis=0)
    return e * (1.0 / jnp.sum(e, axis=1, keepdims=True))


def _features_bwd(phi, dphi):
    t = phi * dphi
    dp = t - phi * jnp.sum(t, axis=1, keepdims=True)
    return (dp[:4] - dp[4:]).reshape(128, phi.shape[2])


def _split_state(acc):
    shape = (128 + XR, 256)
    row, col = _iota(shape, 0), _iota(shape, 1)
    own = jnp.where(row < 128, row // DH, (row - 128) // 8) == (col % 128) // DH
    acc = jnp.where(own, acc, 0.0)
    z8 = acc[128:136] + acc[136:144] + acc[144:152] + acc[152:160]
    zb = jnp.concatenate([z8] * 16, axis=0).T
    return acc.astype(BF), acc[:128].T.astype(BF), zb


def _kernel(x_h, wqkv_h, wphi_ref, wo_h, w1_h, w2_h, go_h,
            out_h, dx_h, dwqkv_h, dwphi_ref, dwo_h, dw1_h, dw2_h,
            x_s, go_s, xn_s, xnT_s, w_s, phi_s, wqT_s, wkvT_s, wo_s, w1_s, w2_s,
            h_s, vT_s, fk_s, dm_s, ds_s, oT_s, dq_s, dkv_s,
            acc_s, st_s, stT_s, zb_s, tile_s, dw1_s,
            x_sem, w_sem, w1_sem, misc_sem, tile_sem, dw1_sem, dw2_sem, dw_sem):

    def rows(i):
        return pl.ds(pl.multiple_of(i * T, T), T)

    def cols(c, n):
        return pl.ds(pl.multiple_of(c * n, n), n)

    def x_copy(i):
        return pltpu.make_async_copy(x_h.at[0, rows(i)], x_s.at[rows(i)], x_sem.at[i])

    def w_copy(j, g):
        return pltpu.make_async_copy(wqkv_h.at[:, cols(j * G + g, 128)], w_s.at[j, g], w_sem.at[j])

    def w1_copy(c):
        return pltpu.make_async_copy(w1_h.at[:, cols(c, FC)], w1_s.at[c], w1_sem.at[0])

    def w2_copy(c):
        return pltpu.make_async_copy(w2_h.at[cols(c, FC)], w2_s.at[c], misc_sem.at[0])

    wo_copy = pltpu.make_async_copy(wo_h, wo_s, misc_sem.at[1])
    go_copy = pltpu.make_async_copy(go_h.at[0], go_s, misc_sem.at[2])
    dwo_copy = pltpu.make_async_copy(wo_s, dwo_h, misc_sem.at[3])

    def tile_copy(dst, i):
        return pltpu.make_async_copy(tile_s.at[i % 2], dst.at[0, rows(i)], tile_sem.at[i % 2])

    def dw1_copy(c):
        return pltpu.make_async_copy(dw1_s.at[c % 2], dw1_h.at[:, cols(c, FC)], dw1_sem.at[c % 2])

    def dw2_copy(c):
        return pltpu.make_async_copy(w2_s.at[c], dw2_h.at[cols(c, FC)], dw2_sem.at[0])

    def dw_copy(j, g):
        return pltpu.make_async_copy(w_s.at[j, g], dwqkv_h.at[:, cols(j * G + g, 128)], dw_sem.at[0])

    for j in (1, 2):
        for g in range(G):
            w_copy(j, g).start()
    x_copy(0).start()
    for c in range(NC):
        w1_copy(c).start()
    for i in range(1, NT):
        x_copy(i).start()
    for g in range(G):
        w_copy(0, g).start()
    for c in range(NC):
        w2_copy(c).start()
    wo_copy.start()
    go_copy.start()

    row, col = _iota((128, 128), 0), _iota((128, 128), 1)
    diag = (row // DH) == (col // DH)
    spread = jnp.where(_iota((DH, 128), 0) == _iota((DH, 128), 1) % DH, 1.0, 0.0).astype(BF)
    for g in range(G):
        blk = jnp.where(diag, _nn(wphi_ref[4 * g:4 * g + 4].reshape(128, DH), spread), 0.0)
        phi_s[0, g] = blk.astype(BF)
        phi_s[1, g] = blk.T.astype(BF)
    acc_s[...] = jnp.zeros(acc_s.shape, F32)

    for g in range(G):
        w_copy(1, g).wait()

    @pl.loop(0, G)
    def _(g):
        wkvT_s[g, :128] = _nt(phi_s[1, g], w_s[1, g]).astype(BF)

    for g in range(G):
        w_copy(2, g).wait()

    @pl.loop(0, G)
    def _(g):
        eye = jnp.where(_iota((128, 128), 0) == _iota((128, 128), 1), 1.0, 0.0).astype(BF)
        wkvT_s[g, 128:] = _nt(eye, w_s[2, g]).astype(BF)

    for c in range(NC):
        w1_copy(c).wait()

    @pl.loop(0, NT)
    def _(i):
        x_copy(i).wait()
        r = rows(i)
        xn32, _ = _layernorm(x_s[r].astype(F32))
        xn = xn32.astype(BF)
        xn_s[r] = xn
        xnT_s[:, r] = xn.T
        for g in range(G):
            kv = _nt(wkvT_s[g], xn)
            fk = _features(kv[:128]).reshape(256, T).astype(BF)
            vT = kv[128:].astype(BF)
            fk_s[g, :, r] = fk
            vT_s[g, :, r] = vT
            acc_s[g] += _nt(jnp.concatenate([vT, jnp.ones((XR, T), BF)], axis=0), fk)
            if g < NC:
                h = _nn(xn, w1_s[g])
                h_s[g, r] = jnp.where(h == 0.0, -0.0, jnp.maximum(h, 0.0)).astype(BF)

    def finish_state():
        @pl.loop(0, G)
        def _(g):
            st_s[g], stT_s[g], zb_s[g] = _split_state(acc_s[g])
            acc_s[g] = jnp.zeros((128 + XR, 256), F32)

    finish_state()
    for g in range(G):
        w_copy(0, g).wait()

    @pl.loop(0, G)
    def _(g):
        wqT_s[cols(g, 128)] = _nt(phi_s[1, g], w_s[0, g]).astype(BF)

    for c in range(NC):
        w2_copy(c).wait()
    wo_copy.wait()
    go_copy.wait()

    @pl.loop(0, NT)
    def _(i):
        @pl.when(i >= 2)
        def _():
            tile_copy(out_h, i - 2).wait()

        r = rows(i)
        pq = _nt(wqT_s[...], xn_s[r])
        fq, oT, rden, m = [], [], [], None
        for g in range(G):
            f = _features(pq[128 * g:128 * (g + 1)])
            nd = _nn(st_s[g], f.reshape(256, T).astype(BF))
            rd = (1.0 / (nd[128:] + 1e-6)).reshape(4, 1, 8, T)
            o = nd[:128].reshape(4, 4, 8, T) * rd
            fq.append(f)
            oT.append(o)
            rden.append(rd)
            if g < NC:
                part = _nn(h_s[g, r], w2_s[g])
                m = part if m is None else m + part
        ob = jnp.concatenate([o.reshape(128, T) for o in oT], axis=0).astype(BF)
        oT_s[:, r] = ob
        s = _tn(ob, wo_s[...])
        sig = 1.0 / (1.0 + jnp.exp(-m))
        gate = m * sig
        go = go_s[r].astype(F32)
        ds = (go * gate).astype(BF)
        ds_s[r] = ds
        tile_s[i % 2] = (x_s[r].astype(F32) + s * gate).astype(BF)
        dm_s[r] = (go * s * (sig + gate * (1.0 - sig))).astype(BF)
        do = _nt(wo_s[...], ds)
        for g in range(G):
            dnum = do[128 * g:128 * (g + 1)].reshape(4, 4, 8, T) * rden[g]
            dden = -jnp.sum((dnum * oT[g]).reshape(4, DH, T), axis=1, keepdims=True)
            dnb = dnum.reshape(128, T).astype(BF)
            ddb = jnp.broadcast_to(dden, (4, 8, T)).reshape(XR, T).astype(BF)
            f = fq[g]
            acc_s[g] += _nt(jnp.concatenate([dnb, ddb], axis=0), f.reshape(256, T).astype(BF))
            zb = jnp.concatenate([zb_s[g]] * (T // 128), axis=1).reshape(8, DH, T)
            df = _nn(stT_s[g], dnb).reshape(8, DH, T) + zb * jnp.concatenate([dden, dden], axis=0)
            dq_s[g, r] = _features_bwd(f, df).astype(BF).T
        tile_copy(out_h, i).start()

    finish_state()

    def k_side_bwd(g):
        for t in range(S // KT):
            r = slice(t * KT, (t + 1) * KT)
            fk = fk_s[g, :, r]
            zb = jnp.concatenate([zb_s[g]] * (KT // 128), axis=1)
            df = (_nn(stT_s[g], vT_s[g, :, r]) + zb).reshape(8, DH, KT)
            dkv_s[g, r, :128] = _features_bwd(fk.astype(F32).reshape(8, DH, KT), df).astype(BF).T
            dkv_s[g, r, 128:] = _nn(st_s[g, :128], fk).astype(BF).T

    @pl.loop(0, NC)
    def _(c):
        @pl.when(c >= 2)
        def _():
            dw1_copy(c - 2).wait()

        h = h_s[c]
        dm = dm_s[...]
        dh = _nt(dm, w2_s[c])
        bits = lax.bitcast_convert_type(h.astype(F32), jnp.int32)
        dh = (dh * jnp.where(bits > 0, 1.0, jnp.where(bits < 0, 0.5, 0.0))).astype(BF)
        w2_s[c] = _tn(h, dm).astype(BF)
        h_s[c] = dh
        k_side_bwd(c)
        dw1_s[c % 2] = _nn(xnT_s[...], dh).astype(BF)
        dw2_copy(c).start()
        dw1_copy(c).start()

    k_side_bwd(G - 1)
    wo_s[...] = _nn(oT_s[...], ds_s[...]).astype(BF)
    dwo_copy.start()

    @pl.loop(0, G)
    def _(g):
        xnT = xnT_s[...]
        dwq = _nn(xnT, dq_s[g]).astype(BF)
        dwkv = _nn(xnT, dkv_s[g]).astype(BF)
        dwk = dwkv[:, :128]
        dphi = _tn(w_s[0, g], dwq) + _tn(w_s[1, g], dwk)
        own = (_iota((128, 128), 0) // DH) == (_iota((128, 128), 1) // DH)
        gather = jnp.where(_iota((128, DH), 0) % DH == _iota((128, DH), 1), 1.0, 0.0).astype(BF)
        dphi = _nn(jnp.where(own, dphi, 0.0).astype(BF), gather)
        dwphi_ref[pl.ds(4 * g, 4)] = dphi.astype(BF).reshape(4, DH, DH)
        w_s[0, g] = _nn(dwq, phi_s[1, g]).astype(BF)
        w_s[1, g] = _nn(dwk, phi_s[1, g]).astype(BF)
        w_s[2, g] = dwkv[:, 128:]
        for j in range(3):
            dw_copy(j, g).start()

    tile_copy(out_h, NT - 2).wait()
    tile_copy(out_h, NT - 1).wait()

    @pl.loop(0, NT)
    def _(i):
        @pl.when(i >= 2)
        def _():
            tile_copy(dx_h, i - 2).wait()

        r = rows(i)
        dxn = None
        for g in range(G):
            part = _nn(dq_s[g, r], wqT_s[128 * g:128 * (g + 1)]) + _nn(dkv_s[g, r], wkvT_s[g])
            dxn = part if dxn is None else dxn + part
        for c in range(NC):
            dxn = dxn + _nt(h_s[c, r], w1_s[c])
        xn, rstd = _layernorm(x_s[r].astype(F32))
        dx = rstd * (dxn - jnp.mean(dxn, axis=-1, keepdims=True)
                     - xn * jnp.mean(dxn * xn, axis=-1, keepdims=True))
        tile_s[i % 2] = (go_s[r].astype(F32) + dx).astype(BF)
        tile_copy(dx_h, i).start()

    for c in range(NC):
        dw2_copy(c).wait()
    dw1_copy(NC - 2).wait()
    dw1_copy(NC - 1).wait()
    dwo_copy.wait()
    for j in range(3):
        for g in range(G):
            dw_copy(j, g).wait()
    tile_copy(dx_h, NT - 2).wait()
    tile_copy(dx_h, NT - 1).wait()


@jax.jit
def pallas_recurrent_scan__linear_kernel_hedgehog__dense_activation_relu__prompt_kernel(
    A_x, A_wqkv, A_w_phi, A_wo, B_x, B_w1, B_w2, grad_out,
):
    del B_x
    hbm = pl.BlockSpec(memory_space=pl.ANY)
    vmem = pl.BlockSpec(memory_space=pltpu.VMEM)
    sds, buf, sem = jax.ShapeDtypeStruct, pltpu.VMEM, pltpu.SemaphoreType.DMA
    return pl.pallas_call(
        _kernel,
        in_specs=[hbm, hbm, vmem, hbm, hbm, hbm, hbm],
        out_specs=[hbm, hbm, hbm, vmem, hbm, hbm, hbm],
        out_shape=[sds(a.shape, BF) for a in (A_x, A_x, A_wqkv, A_w_phi, A_wo, B_w1, B_w2)],
        scratch_shapes=[
            buf((S, D), BF), buf((S, D), BF), buf((S, D), BF), buf((D, S), BF),
            buf((3, G, D, 128), BF), buf((2, G, 128, 128), BF),
            buf((D, D), BF), buf((G, 256, D), BF),
            buf((D, D), BF), buf((NC, D, FC), BF), buf((NC, FC, D), BF),
            buf((NC, S, FC), BF), buf((G, 128, S), BF), buf((G, 256, S), BF),
            buf((S, D), BF), buf((S, D), BF), buf((D, S), BF),
            buf((G, S, 128), BF), buf((G, S, 256), BF),
            buf((G, 128 + XR, 256), F32), buf((G, 128 + XR, 256), BF),
            buf((G, 256, 128), BF), buf((G, 256, 128), F32),
            buf((2, T, D), BF), buf((2, D, FC), BF),
            sem((NT,)), sem((3,)), sem((1,)), sem((4,)), sem((2,)), sem((2,)), sem((1,)), sem((1,)),
        ],
        compiler_params=pltpu.CompilerParams(vmem_limit_bytes=126 * 1024 * 1024),
    )(A_x, A_wqkv, A_w_phi, A_wo, B_w1, B_w2, grad_out)
```

```python
import jax
import jax.numpy as jnp
from jax import lax
import jax.experimental.pallas as pl
import jax.experimental.pallas.tpu as pltpu

S, D, F, H, DH = 2048, 1024, 3584, 32, 32
G = 8
T = 256
NT = S // T
D2, F2, S2 = D // 2, F // 2, S // 2
FC = 256
NC = F2 // FC
PART = ((0, 768), (768, F2 - 768))
KT = 512
XR = 16
BF, F32 = jnp.bfloat16, jnp.float32


def _nn(a, b):
    return lax.dot_general(a, b, (((1,), (0,)), ((), ())), preferred_element_type=F32)


def _nt(a, b):
    return lax.dot_general(a, b, (((1,), (1,)), ((), ())), preferred_element_type=F32)


def _tn(a, b):
    return lax.dot_general(a, b, (((0,), (0,)), ((), ())), preferred_element_type=F32)


def _iota(shape, axis):
    return lax.broadcasted_iota(jnp.int32, shape, axis)


def _layernorm(x):
    xc = x - jnp.mean(x, axis=-1, keepdims=True)
    rstd = lax.rsqrt(jnp.mean(xc * xc, axis=-1, keepdims=True) + 1e-5)
    return xc * rstd, rstd


def _cat(xs, axis=0):
    return jnp.concatenate(xs, axis=axis)


def _features(p):
    p = p.reshape(4, DH, p.shape[1])
    pos = jnp.exp(p - jnp.max(p, axis=1, keepdims=True))
    neg = jnp.exp(jnp.min(p, axis=1, keepdims=True) - p)
    e = _cat([pos[:2], neg[:2], pos[2:], neg[2:]])
    return e * (1.0 / jnp.sum(e, axis=1, keepdims=True))


def _features_bwd(phi, dphi):
    t = phi * dphi
    dp = t - phi * jnp.sum(t, axis=1, keepdims=True)
    return _cat([dp[0:2] - dp[2:4], dp[4:6] - dp[6:8]]).reshape(128, phi.shape[2])


def _split_state(acc, k):
    row, col = _iota(acc.shape, 0), _iota(acc.shape, 1)
    acc = jnp.where(jnp.where(row < 64, row // DH, (row - 64) // 8) == (col % 64) // DH, acc, 0.0)
    zero = jnp.zeros((64, 128), F32)
    val = _cat([acc[:64], zero] if k == 0 else [zero, acc[:64]])
    return acc.astype(BF), val.T.astype(BF), _cat([acc[64:72] + acc[72:80]] * 16).T


A_OP = (((1, 0), (1, 3)), ((1, 2), (1, 3)), ((1, 0),), ((1, 3),), ((1, 0), (1, 1)), ((1, 2), (-1, 0)), ((1, 1), (-1, 3)))
B_OP = (((1, 0), (1, 3)), ((1, 0),), ((1, 1), (-1, 3)), ((1, 2), (-1, 0)), ((1, 3),), ((1, 0), (1, 1)), ((1, 2), (1, 3)))
G_OP = (((1, 0), (1, 3)), ((1, 2), (-1, 3)), ((1, 1), (1, 3)), ((1, 0), (1, 2)), ((1, 1), (-1, 0)), ((1, 3),), ((1, 0),))
Y_ORDER, DA_ORDER, DB_ORDER = (2, 3, 1, 4, 0, 5, 6), (5, 6, 1, 4, 0, 2, 3), (5, 6, 2, 3, 0, 1, 4)


def _signed_sum(terms):
    terms = sorted(terms, key=lambda t: -t[0])
    acc = terms[0][1]
    for sign, x in terms[1:]:
        acc = acc + x if sign > 0 else acc - x
    return acc


def _operand(table, blocks, r):
    if len(table[r]) == 1:
        return blocks[table[r][0][1]].astype(BF)
    return _signed_sum([(sign, blocks[q].astype(F32)) for sign, q in table[r]]).astype(BF)


def _operands(table, blocks):
    return [_operand(table, blocks, r) for r in range(7)]


def _quads(x):
    m, n = x.shape[0] // 2, x.shape[1] // 2
    return x[:m, :n], x[:m, n:], x[m:, :n], x[m:, n:]


def _strassen(table, order, product, emit=None, operand=None, between=None):
    prods, out, nxt = {}, {}, operand and operand(order[0])
    for e, r in enumerate(order):
        prods[r] = product(r, nxt) if operand else product(r)
        if operand and e < 6:
            nxt = operand(order[e + 1])
        for q in range(4):
            terms = [(sign, k) for k in order for sign, b in table[k] if b == q]
            if terms[-1][1] == r:
                out[q] = _signed_sum([(sign, prods[k]) for sign, k in terms])
                if emit:
                    emit(q, out[q])
        if between:
            between(e)
    return out


def _halves(x):
    n = x.shape[0] // T
    return tuple(_cat([x[i * T + o:i * T + o + 128] for i in range(n)]) for o in (0, 128))


def _tiles(top, bot, axis=0):
    return _cat([lax.slice_in_dim(y, i, i + 128, axis=axis)
                 for i in range(0, top.shape[axis], 128) for y in (top, bot)], axis)


B_SLOT = (1, 2, 3, 4)


def _kernel(x_h, wqkv_h, wphi_ref, wo_h, w1_h, w2_h, go_h,
            out_h, dx_h, dwqkv_h, dwphi_ref, dwo_h, dw1_h, dw2_h,
            x_s, go_s, w_s, phi_s, wb_s, wo_s, w1_s, w2_s,
            h_s, vT_s, fk_s, aT_s, gm_s, oT_s, dqkv_s,
            acc_s, st_s, stT_s, zb_s, tile_s, rd_s,
            x_sem, w_sem, misc_sem, tile_sem, dw1_sem, dw_sem):

    def blk(i, n, off=0, size=None):
        return pl.ds(pl.multiple_of(i * n + off, 128), size or n)

    def sub(i, off=0):
        return pl.ds(pl.multiple_of(i * 16 + off, 16), 16)

    def hidden_blocks(r, c):
        (b11, b21), (b12, b22) = _halves(h_s[r, c(0)]), _halves(h_s[r, c(F2)])
        return b11, b12, b21, b22

    def x_copy(p):
        return pltpu.make_async_copy(x_h.at[0, blk(p, 2 * T)], x_s.at[blk(p, 2 * T)], x_sem.at[p])

    def w_raw(j):
        return w_s.at[j] if j < 2 else wo_s

    def w_copies(js, u, sem):
        return [pltpu.make_async_copy(wqkv_h.at[:, blk(u, 256, j * D + o)], w_raw(j).at[:, blk(u, 256, o)], sem)
                for j in js for o in (0, D2)]

    def w1_copies(u):
        return [pltpu.make_async_copy(w1_h.at[blk(q // 2, D2), blk(q % 2, F2, *PART[u])],
                                      w1_s.at[B_SLOT[q], :, pl.ds(*PART[u])], misc_sem.at[u]) for q in range(4)]

    wkv_copies = [w_copies((1, 2), u, w_sem.at[u]) for u in range(2)]
    late_copies = w_copies((0,), 0, w_sem.at[2]) + w_copies((0,), 1, w_sem.at[2]) + [
        pltpu.make_async_copy(w2_h.at[blk(q, F2)], dqkv_s.at[q, blk(0, F2)], w_sem.at[2]) for q in range(2)]
    wo_copy = pltpu.make_async_copy(wo_h, wo_s, misc_sem.at[2])
    go_copy = pltpu.make_async_copy(go_h.at[0], go_s, misc_sem.at[3])
    dwo_copy = pltpu.make_async_copy(wo_s, dwo_h, misc_sem.at[4])

    def tile_copy(dst, i):
        return pltpu.make_async_copy(tile_s.at[i % 2], dst.at[0, blk(i, T)], tile_sem.at[i % 2])

    def fold(j, n, dst):
        lo, hi = [_nt(phi_s[g if j < 2 else G], w_raw(j)[:, blk(g, 128)]) for g in (n, n + 4)]
        return dst, _operands(B_OP, (lo[:, :D2], hi[:, :D2], lo[:, D2:], hi[:, D2:]))

    def put(ref, r, ops):
        for k in range(7):
            ref[k, r] = ops[k]

    def project(rows, p, between=None):
        y = _strassen(G_OP, Y_ORDER, lambda k: _nn(wb_s[k, rows], aT_s[k, :, blk(p, T)]), between=between)
        return _tiles(y[0], y[2], 1), _tiles(y[1], y[3], 1)

    def finish_state():
        for g in range(G):
            for k in range(2):
                r = slice(128 * k, 128 * (k + 1))
                st_s[g, k], stT_s[g, r], zb_s[g, r] = _split_state(acc_s[g, k], k)
                acc_s[g, k] = jnp.zeros((64 + XR, 128), F32)

    def accumulate(g, val, extra, f):
        for k in range(2):
            lhs = _cat([val[64 * k:64 * (k + 1)], extra[XR * k:XR * (k + 1)]])
            acc_s[g, k] += _nt(lhs, f[128 * k:128 * (k + 1)])

    x_copy(0).start()

    row, col = _iota((128, 128), 0), _iota((128, 128), 1)
    spread = jnp.where(_iota((DH, 128), 0) == _iota((DH, 128), 1) % DH, 1.0, 0.0).astype(BF)
    for g in range(G):
        full = _nn(wphi_ref[4 * g:4 * g + 4].reshape(128, DH), spread)
        phi_s[g] = jnp.where((row // DH) == (col // DH), full, 0.0).T.astype(BF)
    phi_s[G] = jnp.where(row == col, 1.0, 0.0).astype(BF)
    x_copy(1).start()
    acc_s[...] = jnp.zeros(acc_s.shape, F32)

    def fq(g, p):
        return dqkv_s.at[1 + p // 2, blk(g, 256), blk(p % 2, 2 * T)]

    def forward():
        @pl.loop(0, NT // 2)
        def _(p):
            x_copy(p).wait()
            for e, copies in enumerate(([x_copy(2), x_copy(3)] + wkv_copies[0], w1_copies(0))):
                @pl.when(p == e)
                def _():
                    for c in copies:
                        c.start()

            @pl.loop(2 * p, 2 * p + 2)
            def _(i):
                ops = []
                for e in range(8):
                    top, bot = [_layernorm(x_s[sub(e, i * T + t)].astype(F32))[0] for t in (0, 128)]
                    ops.append(_operands(A_OP, _quads(_cat([top, bot]))))
                for k in range(7):
                    a = _cat([o[k] for o in ops])
                    gm_s[k, blk(i, 128)] = a
                    aT_s[k, :, blk(i, 128)] = a.T

        for u in range(2):
            for c in wkv_copies[u]:
                c.wait()

            @pl.loop(0, 2)
            def _(e):
                for j in (1, 2):
                    put(wb_s, *fold(j, 2 * u + e, blk(e, 128, D2 * u + 256 * (j + 1))))

            for c in w1_copies(u) + (late_copies if u else []):
                c.wait()
            if u == 0:
                for c in [*wkv_copies[1], *w1_copies(1), *late_copies, go_copy]:
                    c.start()
            else:
                wo_copy.start()
            half = pl.ds(*PART[u])

            @pl.loop(0, D2 // 128)
            def _(i):
                for t in range(8):
                    ops = _operands(B_OP, [w1_s[q, sub(8 * i + t), half] for q in B_SLOT])
                    for k in (0, 2, 3, 5, 6):
                        w1_s[k, sub(8 * i + t), half] = ops[k]

            @pl.loop(0, NT // 2)
            def _(p):
                r = blk(p, 2 * T)

                def prepare(e):
                    for t in range(2 * u):
                        c = sub(2 * e + t, p * (F2 // 4))
                        put(w2_s, c, _operands(B_OP, [dqkv_s[q // 2, c, blk(q % 2, D2)] for q in range(4)]))

                kv = project(slice(D2 * (u + 1), D2 * (u + 2)), p, prepare)

                def k_side(e):
                    prepare(7 + e)
                    if u == 1 and e == 4:
                        put(wb_s, *fold(0, p, blk(p, 128)))
                    if e < 4:
                        g, y = 2 * u + e % 2 + 4 * (e // 2), kv[e // 2][128 * (e % 2):]
                        fk = _features(y[:128]).reshape(256, 2 * T).astype(BF)
                        vT = y[256:384].astype(BF)
                        fk_s[g, :, r] = fk
                        vT_s[g, :, r] = vT
                        accumulate(g, vT, jnp.ones((2 * XR, 2 * T), BF), fk)

                def relu(q, h):
                    h = jnp.where(h == 0.0, -0.0, jnp.maximum(h, 0.0)).astype(BF)
                    for t in range(2):
                        h_s[blk(2 * p + t, T, q // 2 * 128, 128), blk(q % 2, F2, *PART[u])] = h[128 * t:128 * (t + 1)]

                _strassen(G_OP, Y_ORDER, lambda k: _nn(gm_s[k, blk(p, T)], w1_s[k, :, half]), relu, between=k_side)

        finish_state()

        @pl.loop(0, NT)
        def _(n):
            p, u = n // 2, n % 2
            r = blk(p, 2 * T)
            pq = _cat(project(blk(u, 256), p))
            h = hidden_blocks(r, lambda o: slice(o, o + F2))

            def q_side(e):
                if e < 4:
                    g = 2 * u + e % 2 + 4 * (e // 2)
                    f = _features(pq[128 * e:128 * (e + 1)]).reshape(256, 2 * T).astype(BF)
                    nd = [_nn(st_s[g, t], f[128 * t:128 * (t + 1)]) for t in range(2)]
                    rd = 1.0 / (_cat([y[64:] for y in nd]) + 1e-6)
                    o = _cat([y[:64] for y in nd]).reshape(4, 4, 8, 2 * T) * rd.reshape(4, 1, 8, 2 * T)
                    fq(g, p)[...] = f
                    rd_s[g, :, r] = rd
                    oT_s[blk(g, 128), r] = o.reshape(128, 2 * T).astype(BF)

            def keep(q, m):
                gm_s[q, blk(p, T), blk(u, 256)] = m.astype(BF)

            _strassen(G_OP, Y_ORDER, lambda k, a: _nn(a, w2_s[k, :, blk(u, 256)]), keep,
                      lambda k: _operand(A_OP, h, k), q_side)

        wo_copy.wait()
        go_copy.wait()

        @pl.loop(0, NT)
        def _(i):
            @pl.when(i >= 2)
            def _():
                tile_copy(out_h, i - 2).wait()

            r = blk(i, T)
            ob = oT_s[:, r]
            o_t = ob.T
            s, late = [], []
            for u in range(4):
                cols = [slice(128 * u + o, 128 * (u + 1) + o) for o in (0, D2)]
                s.append(_nn(o_t, _cat([wo_s[:, y] for y in cols], 1)))
                m = _cat([_cat([gm_s[2 * t + q, blk(i, 128), cols[0]] for q in range(2)], 1) for t in range(2)])
                m = m.astype(F32)
                x, go = [_cat([z[r, y] for y in cols], 1) for z in (x_s, go_s)]
                sig = 1.0 / (1.0 + jnp.exp(-m))
                act = m * sig
                late.append((cols, x, act, (go, sig), (go.astype(F32) * act).astype(BF)))
            ds = _cat([y[4][:, o:o + 128] for o in (0, 128) for y in late], 1)
            go_s[r] = ds
            for u in range(4):
                cols, x, act, (go, sig), _ = late[u]
                out = (x.astype(F32) + s[u] * act).astype(BF)
                tile_s[i % 2, :, cols[0]], tile_s[i % 2, :, cols[1]] = out[:, :128], out[:, 128:]
                for k, y in enumerate(_operands(G_OP, _quads(s[u] * go.astype(F32) * (sig + act * (1.0 - sig))))):
                    gm_s[k, blk(i, 128), cols[0]] = y
                c = slice(256 * u, 256 * (u + 1))
                dnum = _nt(wo_s[c], ds).reshape(8, 4, 8, T) * rd_s[2 * u:2 * u + 2, :, r].reshape(8, 1, 8, T)
                dnum = dnum.reshape(8, DH, T)
                dden = -jnp.sum(dnum * ob[c].astype(F32).reshape(8, DH, T), axis=1, keepdims=True)
                rd_s[2 * u:2 * u + 2, :, r] = jnp.broadcast_to(dden, (8, 8, T)).reshape(2, 2 * XR, T)
                x_s[r, c] = dnum.reshape(256, T).astype(BF)
            tile_copy(out_h, i).start()

    forward()

    def backward():
        def dw1_copies(c):
            return [pltpu.make_async_copy(gm_s.at[c, :, blk(q, FC)], dw1_h.at[:, blk(c, FC, q * F2)], dw1_sem.at[0])
                    for q in range(2)]

        def dw2_copies(c):
            return [pltpu.make_async_copy(tile_s.at[q], dw2_h.at[blk(c, FC, q * F2)], tile_sem.at[q])
                    for q in range(2)]

        def dw_copy(j, g, n=128):
            return pltpu.make_async_copy(w_s.at[j, :, blk(g, n)], dwqkv_h.at[:, blk(g, n, j * D)], dw_sem.at[j])

        def dwv_copy(u, q):
            r, o = blk(q // 2, D2), q % 2 * D2
            return pltpu.make_async_copy(oT_s.at[r, blk(u, 256, o)], dwqkv_h.at[r, blk(u, 256, 2 * D + o)],
                                         dw_sem.at[2])

        def k_side_bwd(g, t):
            r = blk(t, KT)
            fk = fk_s[g, :, r]
            df = (_nn(stT_s[g], vT_s[g, :, r]) + _cat([zb_s[g]] * (KT // 128), 1)).reshape(8, DH, KT)
            dqkv_s[1, r, blk(g, 128)] = _features_bwd(fk.astype(F32).reshape(8, DH, KT), df).astype(BF).T
            dv = _cat([_nn(st_s[g, k, :64], fk[128 * k:128 * (k + 1)]) for k in range(2)])
            dqkv_s[2, r, blk(g, 128)] = dv.astype(BF).T

        def q_side_bwd(g, t):
            r = blk(t, KT)
            dnum = _cat([x_s[blk(2 * t + e, T, g % 2 * 128, 128), blk(g // 2, T)] for e in range(2)], 1)
            dden, f = rd_s[g, :, r], fq(g, t)[...]
            accumulate(g, dnum, dden.astype(BF), f)
            dden = dden.reshape(4, 1, 8, KT)
            zb = _cat([zb_s[g]] * (KT // 128), 1).reshape(8, 4, 8, KT)
            df = _nn(stT_s[g], dnum).reshape(8, 4, 8, KT) + zb * _cat([dden[:2], dden[:2], dden[2:], dden[2:]])
            dq = _features_bwd(f.astype(F32).reshape(8, DH, KT), df.reshape(8, DH, KT))
            dqkv_s[0, r, blk(g, 128)] = dq.astype(BF).T

        def wo_grad(half, side):
            @pl.loop(0, 2)
            def _(t):
                c = blk(t, 256, half * D2)
                for e in range(2):
                    wo_s[blk(e, D2), c] = _nn(oT_s[blk(e, D2)], go_s[:, c]).astype(BF)
                    if e == 0:
                        side(G - 1, 2 * t)
                        side(G - 1, 2 * t + 1)

        wo_grad(0, q_side_bwd)

        @pl.loop(0, NC)
        def _(c):
            def drain(e):
                if e == 1:
                    for cp in dw2_copies(c):
                        cp.wait()

            def keep(q, y):
                tile_s[q // 2, :, blk(q % 2, D2)] = y.astype(BF)

            h = hidden_blocks(slice(None), lambda o: blk(c, FC, o))
            _strassen(B_OP, (2, 3, 5, 6, 0, 1, 4), lambda k, aT: _nn(aT, gm_s[k]), keep,
                      lambda k: _operand(A_OP, h, k).T, drain)
            for cp in dw2_copies(c):
                cp.start()

        @pl.loop(0, NC)
        def _(c):
            for v in range(2):
                def keep(q, y):
                    for t in range(NT // 2):
                        r, cc = blk(4 * v + t, T, q // 2 * 128, 128), blk(c, FC, q % 2 * F2)
                        bits = lax.bitcast_convert_type(h_s[r, cc].astype(F32), jnp.int32)
                        slope = jnp.where(bits > 0, 1.0, jnp.where(bits < 0, 0.5, 0.0))
                        h_s[r, cc] = (y[128 * t:128 * (t + 1)] * slope).astype(BF)

                _strassen(A_OP, DA_ORDER, lambda k: _nt(gm_s[k, blk(v, S2 // 2)], w2_s[k, blk(c, FC)]), keep,
                          between=lambda e: q_side_bwd(c, 2 * v + e // 3) if e in (0, 3) else None)

        finish_state()
        wo_grad(1, k_side_bwd)
        for cp in [dwo_copy, go_copy] + [x_copy(p) for p in range(NT // 2)]:
            cp.start()

        @pl.loop(0, NC)
        def _(c):
            def keep(q, y):
                gm_s[c, blk(q // 2, D2), blk(q % 2, FC)] = y.astype(BF)

            dh = hidden_blocks(slice(None), lambda o: blk(c, FC, o))
            _strassen(B_OP, DB_ORDER, lambda k, g: _nn(aT_s[k], g), keep, lambda k: _operand(G_OP, dh, k),
                      lambda e: k_side_bwd(c, (0, 1, 4, 5).index(e)) if e in (0, 1, 4, 5) else None)
            for cp in dw1_copies(c):
                cp.start()

        for cp in dw2_copies(NC - 1):
            cp.wait()

        def projection_grad(j, u, between=None):
            (g11, g21), (g12, g22) = [_halves(dqkv_s[j, :, blk(u, 256, o)]) for o in (0, D2)]

            def keep(q, y):
                oT_s[blk(q // 2, D2), blk(u, 256, j % 2 * D + q % 2 * D2)] = y.astype(BF)
                if between:
                    dwv_copy(u, q).start()

            _strassen(B_OP, DB_ORDER, lambda k, g: _nn(aT_s[k], g), keep,
                      lambda k: _operand(G_OP, (g11, g12, g21, g22), k), between)

        @pl.loop(0, 4)
        def _(n):
            projection_grad(n // 2, n % 2)

        for c in range(NC):
            for cp in dw1_copies(c):
                cp.wait()
        for cp in [go_copy] + [x_copy(p) for p in range(NT // 2)]:
            cp.wait()

        def norm_grad(i):
            return _cat([_cat([gm_s[2 * t + q, blk(i, 128)] for q in range(2)], 1) for t in range(2)])

        def norm_bwd(i, e, dxn):
            r, dxn = sub(e, i * T), dxn[16 * e:16 * (e + 1)].astype(F32)
            xn, rstd = _layernorm(x_s[r].astype(F32))
            dx = rstd * (dxn - jnp.mean(dxn, axis=-1, keepdims=True)
                         - xn * jnp.mean(dxn * xn, axis=-1, keepdims=True))
            tile_s[i % 2, sub(e)] = (go_s[r].astype(F32) + dx).astype(BF)

        @pl.loop(0, NT)
        def _(n):
            @pl.when(n >= 4)
            def _():
                tile_copy(dx_h, n - 4).wait()

            p, u = n // 2, n % 2
            r, c = blk(p, 2 * T), blk(n, 128)
            dh = hidden_blocks(r, lambda o: slice(o, o + F2))
            (g11, g21), (g12, g22) = [
                _halves(_cat([dqkv_s[0, r, o:o + D2]] + [dqkv_s[j, r, o + t:o + t + 256]
                                                         for t in (0, 256) for j in (1, 2)], 1)) for o in (0, D2)]
            dphi, dxn = [], []

            def extra(e):
                if e == 0:
                    dxn.append(norm_grad(jnp.maximum(n - 2, 0)))
                for t in range(3 * e, min(3 * e + 3, 16)):
                    norm_bwd(jnp.maximum(n - 2, 0), t, dxn[0])
                if e in (2, 3):
                    dw = oT_s[:, blk(n, 128, (e - 2) * D)]
                    dphi.append(_tn(w_s[e - 2, :, c], dw))
                    for t in range(0, D, 256):
                        w_s[e - 2, t:t + 256, c] = _nn(dw[t:t + 256], phi_s[n]).astype(BF)
                if e == 4:
                    own = (_iota((128, 128), 0) // DH) == (_iota((128, 128), 1) // DH)
                    gather = jnp.where(_iota((128, DH), 0) % DH == _iota((128, DH), 1), 1.0, 0.0).astype(BF)
                    y = _nn(jnp.where(own, dphi[0] + dphi[1], 0.0).astype(BF), gather)
                    dwphi_ref[pl.ds(4 * n, 4)] = y.astype(BF).reshape(4, DH, DH)

            def keep(q, y):
                gm_s[q, blk(p, T), blk(u, 256)] = y.astype(BF)

            _strassen(A_OP, DA_ORDER,
                      lambda k, g: _nt(g[0], w1_s[k, blk(u, 256)]) + _nn(g[1], wb_s[k, :, blk(u, 256)]), keep,
                      lambda k: (_operand(G_OP, dh, k), _operand(G_OP, (g11, g12, g21, g22), k)), extra)
            dw_copy(0, n).start()
            dw_copy(1, n).start()

            @pl.when(n >= 2)
            def _():
                tile_copy(dx_h, n - 2).start()

        @pl.loop(0, 2)
        def _(u):
            dxn = norm_grad(NT - 2 + u)

            def rest(e):
                if e == 0:
                    tile_copy(dx_h, NT - 4 + u).wait()
                if e < 4:
                    for t in range(4):
                        norm_bwd(NT - 2 + u, 4 * e + t, dxn)
                if e == 4:
                    tile_copy(dx_h, NT - 2 + u).start()

            projection_grad(2, u, rest)

        for n in range(8):
            dwv_copy(n // 4, n % 4).wait()
        dwo_copy.wait()
        for j in range(2):
            dw_copy(j, 0, D).wait()
        tile_copy(dx_h, NT - 2).wait()
        tile_copy(dx_h, NT - 1).wait()

    backward()


@jax.jit
def pallas_recurrent_scan__linear_kernel_hedgehog__dense_activation_relu__prompt_kernel(
    A_x, A_wqkv, A_w_phi, A_wo, B_x, B_w1, B_w2, grad_out,
):
    del B_x
    hbm = pl.BlockSpec(memory_space=pl.ANY)
    vmem = pl.BlockSpec(memory_space=pltpu.VMEM)
    sds, buf, sem = jax.ShapeDtypeStruct, pltpu.VMEM, pltpu.SemaphoreType.DMA
    return pl.pallas_call(
        _kernel,
        in_specs=[hbm, hbm, vmem, hbm, hbm, hbm, hbm],
        out_specs=[hbm, hbm, hbm, vmem, hbm, hbm, hbm],
        out_shape=[sds(a.shape, BF) for a in (A_x, A_x, A_wqkv, A_w_phi, A_wo, B_w1, B_w2)],
        scratch_shapes=[
            buf((S, D), BF), buf((S, D), BF),
            buf((2, D, D), BF), buf((G + 1, 128, 128), BF), buf((7, 3 * D2, D2), BF),
            buf((D, D), BF), buf((7, D2, F2), BF), buf((7, F2, D2), BF),
            buf((S, F), BF), buf((G, 128, S), BF), buf((G, 256, S), BF),
            buf((7, D2, S2), BF), buf((7, S2, D2), BF),
            buf((D, S), BF), buf((3, S, D), BF),
            buf((G, 2, 64 + XR, 128), F32), buf((G, 2, 64 + XR, 128), BF),
            buf((G, 256, 128), BF), buf((G, 256, 128), F32), buf((2, T, D), BF), buf((G, 2 * XR, S), F32),
            sem((4,)), sem((3,)), sem((5,)), sem((2,)), sem((1,)), sem((3,)),
        ],
        compiler_params=pltpu.CompilerParams(flags={"XLA_TPU_EVENLY_DISTRIBUTE_CRITICAL_NODES": True}, vmem_limit_bytes=128 * 1024 * 1024),
    )(A_x, A_wqkv, A_w_phi, A_wo, B_w1, B_w2, grad_out)
```
